```python
import jax
import jax.numpy as jnp

def _softmax(x, axis=-1):
    return jax.nn.softmax(x, axis=axis)
def _gelu(x):
    return jax.nn.gelu(x, approximate=True)
def _silu(x):
    return jax.nn.silu(x)
def _sigmoid(x):
    return jax.nn.sigmoid(x)
def _layernorm(x, axis=-1, eps=1e-5):
    m = jnp.mean(x, axis=axis, keepdims=True)
    v = jnp.var(x, axis=axis, keepdims=True)
    return (x - m) / jnp.sqrt(v + eps)
def _scatter_add(tgt, idx, src, axis=0):
    return tgt.at[idx].add(src)
def _segment_sum(src, seg, n):
    return jax.ops.segment_sum(src, seg, n)
class _Rng:
    def __init__(self, key):
        self._k = key
    def _next(self):
        self._k, sub = jax.random.split(self._k)
        return sub
    def normal(self, shape):
        return jax.random.normal(self._next(), shape, dtype=jnp.bfloat16)
    def randint(self, lo, hi, shape):
        return jax.random.randint(self._next(), shape, lo, hi, dtype=jnp.int32)
    def uniform(self, shape, lo=0.0, hi=1.0):
        return jax.random.uniform(self._next(), shape, jnp.bfloat16, lo, hi)
    def permutation(self, n):
        return jax.random.permutation(self._next(), n)


kernel_name = 'gated_mix__compressed_kv_cla__sliding_block_cached__decode'

def setup_inputs():
    _rng = _Rng(jax.random.key(int.from_bytes(__import__("os").urandom(4), "little")))
    _w = (lambda a: (lambda t: t.astype(jnp.bfloat16) if jnp.issubdtype(t.dtype, jnp.floating) else t)(jnp.asarray(a)))
    def _A_setup():
        B, H, Sq, Sk, D, M = 8, 32, 1, 4096, 128, 512
        Dc = 4 * D
        return {
            "x": _w((lambda *s: _rng.normal(s) * 0.05)(B, Sq, M)),
            "c_kv": _w((lambda *s: _rng.normal(s) * 0.05)(B, Sk, Dc)),
            "w_q": _w((lambda *s: _rng.normal(s) * 0.05)(M, H, D) * (M ** -0.5)),
            "w_uk": _w((lambda *s: _rng.normal(s) * 0.05)(Dc, H, D) * (Dc ** -0.5)),
            "w_uv": _w((lambda *s: _rng.normal(s) * 0.05)(Dc, H, D) * (Dc ** -0.5)),
            "w_o": _w((lambda *s: _rng.normal(s) * 0.05)(H, D, M) * ((H * D) ** -0.5)),
        }
    _A_in = _A_setup()

    def _B_setup():
        B, Sq, D = 8, 1, 512
        Hq, Hkv, Sk, Dh = 32, 8, 4096, 128
        assert Hq % Hkv == 0, (Hq, Hkv)
        return {
            "x": _w((lambda *s: _rng.normal(s) * 0.05)(B, Sq, D)),
            "k_cache": _w((lambda *s: _rng.normal(s) * 0.05)(B, Hkv, Sk, Dh)),
            "v_cache": _w((lambda *s: _rng.normal(s) * 0.05)(B, Hkv, Sk, Dh)),
            "wq": _w((lambda *s: _rng.normal(s) * 0.05)(D, Hq * Dh) * (D ** -0.5)),
            "wo": _w((lambda *s: _rng.normal(s) * 0.05)(Hq * Dh, D) * ((Hq * Dh) ** -0.5)),
        }
    _B_in = _B_setup()

    return {
        "A_x": _A_in["x"],
        "A_c_kv": _A_in["c_kv"],
        "A_w_q": _A_in["w_q"],
        "A_w_uk": _A_in["w_uk"],
        "A_w_uv": _A_in["w_uv"],
        "A_w_o": _A_in["w_o"],
        "B_x": _B_in["x"],
        "B_k_cache": _B_in["k_cache"],
        "B_v_cache": _B_in["v_cache"],
        "B_wq": _B_in["wq"],
        "B_wo": _B_in["wo"],
        "gate_w": _w((lambda *s: _rng.normal(s) * 0.05)(512)),
    }

def reference(A_x, A_c_kv, A_w_q, A_w_uk, A_w_uv, A_w_o, B_x, B_k_cache, B_v_cache, B_wq, B_wo, gate_w):
    def _A_ref(x, c_kv, w_q, w_uk, w_uv, w_o):
        B, Sq, M = x.shape[0], x.shape[1], x.shape[2]
        Sk = c_kv.shape[1]
        H, D = w_q.shape[1], w_q.shape[2]
        q = jnp.einsum("bqm,mhd->bhqd", x, w_q)
        k = jnp.einsum("bkc,chd->bhkd", c_kv, w_uk)
        v = jnp.einsum("bkc,chd->bhkd", c_kv, w_uv)
        scores = jnp.einsum("bhqd,bhkd->bhqk", q, k) * (D ** -0.5)
        off = Sk - Sq
        qi = jnp.arange(Sq)[:, None]
        kj = jnp.arange(Sk)[None, :]
        cmask = kj <= (qi + off)
        scores = jnp.where(cmask[None, None], scores, -1e9)
        p = _softmax(scores, axis=-1)
        ctx = jnp.einsum("bhqk,bhkd->bhqd", p, v)
        return jnp.einsum("bhqd,hdm->bqm", ctx, w_o)

    def _B_ref(x, k_cache, v_cache, wq, wo):
        B, Sq, D = x.shape
        Hq, Dh = 32, 128
        Hkv, Sk = k_cache.shape[1], k_cache.shape[2]
        W = min(4096, max(256, Sk // 4))
        rep = Hq // Hkv
        q = (lambda x, *d: x.transpose(*d))((x @ wq).reshape(B, Sq, Hq, Dh), 0, 2, 1, 3)
        k = jnp.repeat(k_cache[:, :, Sk - W:, :], rep, axis=1)
        v = jnp.repeat(v_cache[:, :, Sk - W:, :], rep, axis=1)
        scores = jnp.einsum("bhqd,bhkd->bhqk", q, k) * (Dh ** -0.5)
        p = _softmax(scores, axis=-1)
        o = jnp.einsum("bhqk,bhkd->bhqd", p, v)
        return (lambda x, *d: x.transpose(*d))(o, 0, 2, 1, 3).reshape(B, Sq, Hq * Dh) @ wo

    x = A_x
    g = _sigmoid((x * gate_w).sum(-1, keepdims=True))
    a = _A_ref(x, A_c_kv, A_w_q, A_w_uk, A_w_uv, A_w_o)
    b = _B_ref(x, B_k_cache, B_v_cache, B_wq, B_wo)
    return g * a + (1 - g) * b
```

```python
import functools
import jax
import jax.numpy as jnp
from jax import lax
from jax.experimental import pallas as pl
from jax.experimental.pallas import tpu as pltpu

B, H, SK, D, M, DC = 8, 32, 4096, 128, 512, 512
HKV, W = 8, 1024
NT = (((1,), (1,)), ((), ()))
NN = (((1,), (0,)), ((), ()))
F32, BF16 = jnp.float32, jnp.bfloat16
NWO = 8
SCALE = float(D) ** -0.5


def _mm(a, b, dims=NN):
    return lax.dot_general(a, b, dims, preferred_element_type=F32)


def _head_pair(w32_ref, j):
    w = w32_ref[pl.ds(j, M, stride=H // 2), :]
    lo = pltpu.bitcast(w << 16, F32).astype(BF16)
    hi = pltpu.bitcast(w & jnp.uint32(0xFFFF0000), F32).astype(BF16)
    return lo, hi


def kernel(x_hbm, gw_hbm, c_hbm, wq_hbm, wuk_hbm, wuv_hbm, wo_hbm, k_hbm, v_hbm, wqb_hbm, wob_hbm,
           o_ref,
           x_v, gw_v, wq_v, wuk_v, wuv_v, wo_v, wqb_v, wob_v, c_v, k_v, v_v,
           q_s, ql_s, cl_s, qb_s, ob_s,
           sem_s, sem_w, sem_o, sem_c, sem_k, sem_v):

    def c_copy(b):
        return pltpu.make_async_copy(c_hbm.at[b], c_v.at[b % 2], sem_c.at[b % 2])

    def k_copy(b):
        return pltpu.make_async_copy(k_hbm.at[b, :, pl.ds(SK - W, W), :], k_v.at[b % 2], sem_k.at[b % 2])

    def v_copy(b):
        return pltpu.make_async_copy(v_hbm.at[b, :, pl.ds(SK - W, W), :], v_v.at[b % 2], sem_v.at[b % 2])

    x_cp = pltpu.make_async_copy(x_hbm, x_v, sem_s.at[0])
    gw_cp = pltpu.make_async_copy(gw_hbm, gw_v, sem_s.at[1])
    wq_cp = pltpu.make_async_copy(wq_hbm, wq_v, sem_w.at[0])
    wuk_cp = pltpu.make_async_copy(wuk_hbm, wuk_v, sem_w.at[1])
    wqb_cp = pltpu.make_async_copy(wqb_hbm, wqb_v, sem_w.at[2])
    wuv_cp = pltpu.make_async_copy(wuv_hbm, wuv_v, sem_w.at[3])
    wo_cp = pltpu.make_async_copy(wo_hbm, wo_v, sem_w.at[4])
    RW = (H * D) // NWO
    wob_cp = [pltpu.make_async_copy(wob_hbm.at[pl.ds(i * RW, RW)], wob_v.at[pl.ds(i * RW, RW)], sem_o.at[i])
              for i in range(NWO)]

    wq_cp.start()
    x_cp.start()
    gw_cp.start()
    wuk_cp.start()
    wqb_cp.start()

    x_cp.wait()
    gw_cp.wait()
    x32 = x_v[...].astype(F32)
    x = x_v[...]

    wq_cp.wait()
    c_copy(0).start()
    wq32 = wq_v.bitcast(jnp.uint32)
    for j in range(H // 2):
        lo, hi = _head_pair(wq32, j)
        q_s[2 * j] = _mm(x, lo)
        q_s[2 * j + 1] = _mm(x, hi)

    wuk_cp.wait()
    k_copy(0).start()
    wuk32 = wuk_v.bitcast(jnp.uint32)
    for j in range(H // 2):
        lo, hi = _head_pair(wuk32, j)
        ql_s[:, 2 * j, :] = _mm(q_s[2 * j].astype(BF16), lo, NT) * SCALE
        ql_s[:, 2 * j + 1, :] = _mm(q_s[2 * j + 1].astype(BF16), hi, NT) * SCALE

    wqb_cp.wait()
    v_copy(0).start()
    for h in range(H):
        qb_s[:, h, :] = _mm(x, wqb_v[:, h * D:(h + 1) * D])

    row = lax.broadcasted_iota(jnp.int32, (8, W), 0)
    rowd = lax.broadcasted_iota(jnp.int32, (8, D), 0)

    def body(b, carry):
        slot = b % 2
        c_copy(b).wait()

        @pl.when(b + 1 < B)
        def _():
            c_copy(b + 1).start()

        @pl.when(b + 1 == B)
        def _():
            wuv_cp.start()

        c = c_v.at[slot]
        s = _mm(ql_s[b].astype(BF16), c[...], NT)
        m = jnp.max(s, axis=-1, keepdims=True)
        e = jnp.exp(s - m)
        l = jnp.sum(e, axis=-1, keepdims=True)
        o = _mm(e.astype(BF16), c[...])
        cl_s[b] = o / l

        k_copy(b).wait()

        @pl.when(b + 1 < B)
        def _():
            k_copy(b + 1).start()

        @pl.when(b + 1 == B)
        def _():
            wo_cp.start()

        v_copy(b).wait()

        @pl.when(b + 1 < B)
        def _():
            v_copy(b + 1).start()

        @pl.when(b + 1 == B)
        def _():
            for cp in wob_cp:
                cp.start()

        qb = qb_s[b].astype(BF16).astype(F32) * SCALE
        for i in range(HKV // 2):
            qi = qb[8 * i:8 * i + 8, :].astype(BF16)
            s0 = _mm(qi, k_v[slot, 2 * i], NT)
            s1 = _mm(qi, k_v[slot, 2 * i + 1], NT)
            sb = jnp.where(row < 4, s0, s1)
            mb = jnp.max(sb, axis=-1, keepdims=True)
            eb = jnp.exp(sb - mb)
            lb = jnp.sum(eb, axis=-1, keepdims=True)
            pb = eb.astype(BF16)
            o0 = _mm(pb, v_v[slot, 2 * i])
            o1 = _mm(pb, v_v[slot, 2 * i + 1])
            ob_s[b, 8 * i:8 * i + 8, :] = jnp.where(rowd < 4, o0, o1) / lb
        return carry

    lax.fori_loop(0, B, body, 0)

    wuv_cp.wait()
    wuv32 = wuv_v.bitcast(jnp.uint32)
    ctx = []
    for j in range(H // 2):
        lo, hi = _head_pair(wuv32, j)
        ctx.append(_mm(cl_s[:, 2 * j, :].astype(BF16), lo).astype(BF16))
        ctx.append(_mm(cl_s[:, 2 * j + 1, :].astype(BF16), hi).astype(BF16))
    ctx = jnp.concatenate(ctx, axis=1)
    wo_cp.wait()
    a = _mm(ctx, wo_v[...])

    ob = jnp.concatenate([ob_s[:, h, :].astype(BF16) for h in range(H)], axis=1)
    g = jax.nn.sigmoid(jnp.sum(x32 * gw_v[...].astype(F32).reshape(1, M), axis=-1, keepdims=True))
    bo = jnp.zeros((B, M), F32)
    for i in range(NWO):
        wob_cp[i].wait()
        bo = bo + _mm(ob[:, i * RW:(i + 1) * RW], wob_v[pl.ds(i * RW, RW), :])
    out = (g * a + (1.0 - g) * bo).astype(o_ref.dtype)
    o_ref[...] = out


@jax.jit
def pallas_gated_mix__compressed_kv_cla__sliding_block_cached__decode_kernel(
    A_x: jax.Array,
    A_c_kv: jax.Array,
    A_w_q: jax.Array,
    A_w_uk: jax.Array,
    A_w_uv: jax.Array,
    A_w_o: jax.Array,
    B_x: jax.Array,
    B_k_cache: jax.Array,
    B_v_cache: jax.Array,
    B_wq: jax.Array,
    B_wo: jax.Array,
    gate_w: jax.Array,
):
    hbm = pl.BlockSpec(memory_space=pltpu.HBM)
    return pl.pallas_call(
        kernel,
        out_shape=jax.ShapeDtypeStruct((B, M), A_x.dtype),
        in_specs=[hbm] * 11,
        out_specs=pl.BlockSpec(memory_space=pltpu.VMEM),
        scratch_shapes=[
            pltpu.VMEM((B, M), BF16),
            pltpu.VMEM((M,), BF16),
            pltpu.VMEM((M * H, D), BF16),
            pltpu.VMEM((DC * H, D), BF16),
            pltpu.VMEM((DC * H, D), BF16),
            pltpu.VMEM((H * D, M), BF16),
            pltpu.VMEM((M, H * D), BF16),
            pltpu.VMEM((H * D, M), BF16),
            pltpu.VMEM((2, SK, DC), BF16),
            pltpu.VMEM((2, HKV, W, D), BF16),
            pltpu.VMEM((2, HKV, W, D), BF16),
            pltpu.VMEM((H, B, D), F32),
            pltpu.VMEM((B, H, DC), F32),
            pltpu.VMEM((B, H, DC), F32),
            pltpu.VMEM((B, H, D), F32),
            pltpu.VMEM((B, H, D), F32),
            pltpu.SemaphoreType.DMA((2,)),
            pltpu.SemaphoreType.DMA((5,)),
            pltpu.SemaphoreType.DMA((NWO,)),
            pltpu.SemaphoreType.DMA((2,)),
            pltpu.SemaphoreType.DMA((2,)),
            pltpu.SemaphoreType.DMA((2,)),
        ],
        compiler_params=pltpu.CompilerParams(vmem_limit_bytes=100 * 1024 * 1024),
    )(A_x.reshape(B, M), gate_w, A_c_kv, A_w_q.reshape(M * H, D), A_w_uk.reshape(DC * H, D), A_w_uv.reshape(DC * H, D),
      A_w_o.reshape(H * D, M), B_k_cache, B_v_cache, B_wq, B_wo).reshape(B, 1, M)
```

```python
import jax
import jax.numpy as jnp
from jax import lax
import jax.experimental.pallas as pl
import jax.experimental.pallas.tpu as pltpu

F32, BF16 = jnp.float32, jnp.bfloat16
N_SEMS = 3

_NN = (((1,), (0,)), ((), ()))
_NT = (((1,), (1,)), ((), ()))


def _mm(a, b, dims=_NN):
    return lax.dot_general(a, b, dims, preferred_element_type=F32)


def _head_pair(w32_ref, j, rows, heads):
    w = w32_ref[pl.ds(j, rows, stride=heads // 2), :]
    even = pltpu.bitcast(w << 16, F32).astype(BF16)
    odd = pltpu.bitcast(w & jnp.uint32(0xFFFF0000), F32).astype(BF16)
    return even, odd


def _exp_max(s):
    e = jnp.exp(s - jnp.max(s, axis=-1, keepdims=True))
    return e, jnp.sum(e, axis=-1, keepdims=True)


def _chunks(total):
    sizes = [total // 4] * 3 + [total // 8, total // 16, total // 32, total // 32]
    assert sum(sizes) == total and all(s % 128 == 0 for s in sizes), sizes
    return sizes


@jax.jit
def pallas_gated_mix__compressed_kv_cla__sliding_block_cached__decode_kernel(
    A_x: jax.Array,
    A_c_kv: jax.Array,
    A_w_q: jax.Array,
    A_w_uk: jax.Array,
    A_w_uv: jax.Array,
    A_w_o: jax.Array,
    B_x: jax.Array,
    B_k_cache: jax.Array,
    B_v_cache: jax.Array,
    B_wq: jax.Array,
    B_wo: jax.Array,
    gate_w: jax.Array,
):
    del B_x
    B, Sq, M = A_x.shape
    _, SK, DC = A_c_kv.shape
    _, H, D = A_w_q.shape
    _, HKV, SKB, _ = B_k_cache.shape
    W = min(4096, max(256, SKB // 4))
    REP = H // HKV
    assert Sq == 1 and B == 8 and REP == 4 and D == 128, (Sq, B, REP, D)
    scale = float(D) ** -0.5
    wob_rows = _chunks(H * D)
    wob_offs = [sum(wob_rows[:i]) for i in range(len(wob_rows))]

    def kernel(x_hbm, gw_hbm, c_hbm, wq_hbm, wuk_hbm, wuv_hbm, wo_hbm,
               k_hbm, v_hbm, wqb_hbm, wob_hbm,
               o_ref,
               x_v, gw_v, wq_v, wuk_v, wuv_v, wo_v, wqb_v, wob_v, c_v, k_v, v_v,
               q_s, qlat_s, clat_s, qb_s, ob_s, sems):

        def c_copy(b):
            return pltpu.make_async_copy(c_hbm.at[b], c_v.at[b % 2], sems.at[0])

        def k_copy(b):
            return pltpu.make_async_copy(
                k_hbm.at[b, :, pl.ds(SKB - W, W), :], k_v.at[b % 2], sems.at[1])

        def v_copy(b):
            return pltpu.make_async_copy(
                v_hbm.at[b, :, pl.ds(SKB - W, W), :], v_v.at[b % 2], sems.at[2])

        x_cp = pltpu.make_async_copy(x_hbm, x_v, sems.at[0])
        gw_cp = pltpu.make_async_copy(gw_hbm, gw_v, sems.at[0])
        wq_cp = pltpu.make_async_copy(wq_hbm, wq_v, sems.at[0])
        wuk_cp = pltpu.make_async_copy(wuk_hbm, wuk_v, sems.at[1])
        wqb_cp = pltpu.make_async_copy(wqb_hbm, wqb_v, sems.at[2])
        tail = [pltpu.make_async_copy(wuv_hbm, wuv_v, sems.at[0]),
                pltpu.make_async_copy(wo_hbm, wo_v, sems.at[1])]
        tail += [pltpu.make_async_copy(wob_hbm.at[pl.ds(o, n)], wob_v.at[pl.ds(o, n)],
                                       sems.at[(2 + i) % N_SEMS])
                 for i, (o, n) in enumerate(zip(wob_offs, wob_rows))]

        def tail_wait(t):
            tail[t].wait()
            if t + N_SEMS < len(tail):
                tail[t + N_SEMS].start()

        wq_cp.start()
        x_cp.start()
        gw_cp.start()
        wuk_cp.start()
        wqb_cp.start()

        x_cp.wait()
        gw_cp.wait()
        wq_cp.wait()
        c_copy(0).start()
        x = x_v[...]

        wq32 = wq_v.bitcast(jnp.uint32)
        for j in range(H // 2):
            for h, w in zip((2 * j, 2 * j + 1), _head_pair(wq32, j, M, H)):
                q_s[h] = _mm(x, w)

        wuk_cp.wait()
        k_copy(0).start()
        wuk32 = wuk_v.bitcast(jnp.uint32)
        for j in range(H // 2):
            for h, w in zip((2 * j, 2 * j + 1), _head_pair(wuk32, j, DC, H)):
                qlat_s[:, h, :] = _mm(q_s[h].astype(BF16), w, _NT) * scale

        wqb_cp.wait()
        v_copy(0).start()
        for h in range(H):
            qb_s[:, h, :] = _mm(x, wqb_v[:, h * D:(h + 1) * D])

        row_w = lax.broadcasted_iota(jnp.int32, (2 * REP, W), 0)
        row_d = lax.broadcasted_iota(jnp.int32, (2 * REP, D), 0)

        def start_next(b, copy, last):
            @pl.when(b + 1 < B)
            def _():
                copy(b + 1).start()

            @pl.when(b + 1 == B)
            def _():
                last.start()

        def per_batch(b, carry):
            slot = b % 2

            c_copy(b).wait()
            start_next(b, c_copy, tail[0])
            c = c_v.at[slot]
            e, l = _exp_max(_mm(qlat_s[b].astype(BF16), c[...], _NT))
            clat_s[b] = _mm(e.astype(BF16), c[...]) / l

            k_copy(b).wait()
            start_next(b, k_copy, tail[1])
            v_copy(b).wait()
            start_next(b, v_copy, tail[2])
            qb = (qb_s[b].astype(BF16).astype(F32) * scale).astype(BF16)
            for i in range(HKV // 2):
                qi = qb[2 * REP * i:2 * REP * (i + 1), :]
                s = jnp.where(row_w < REP,
                              _mm(qi, k_v[slot, 2 * i], _NT),
                              _mm(qi, k_v[slot, 2 * i + 1], _NT))
                eb, lb = _exp_max(s)
                p = eb.astype(BF16)
                o = jnp.where(row_d < REP,
                              _mm(p, v_v[slot, 2 * i]),
                              _mm(p, v_v[slot, 2 * i + 1]))
                ob_s[b, 2 * REP * i:2 * REP * (i + 1), :] = o / lb
            return carry

        lax.fori_loop(0, B, per_batch, 0)

        tail_wait(0)
        wuv32 = wuv_v.bitcast(jnp.uint32)
        ctx = []
        for j in range(H // 2):
            for h, w in zip((2 * j, 2 * j + 1), _head_pair(wuv32, j, DC, H)):
                ctx.append(_mm(clat_s[:, h, :].astype(BF16), w).astype(BF16))
        ctx = jnp.concatenate(ctx, axis=1)
        ob = jnp.concatenate([ob_s[:, h, :].astype(BF16) for h in range(H)], axis=1)
        g = jax.nn.sigmoid(jnp.sum(x.astype(F32) * gw_v[...].astype(F32).reshape(1, M),
                                   axis=-1, keepdims=True))
        tail_wait(1)
        ga = g * _mm(ctx, wo_v[...])

        bo = jnp.zeros((B, M), F32)
        for i, (o, n) in enumerate(zip(wob_offs, wob_rows)):
            tail_wait(2 + i)
            bo = bo + _mm(ob[:, o:o + n], wob_v[pl.ds(o, n), :])

        o_ref[...] = (ga + (1.0 - g) * bo).astype(o_ref.dtype)

    hbm = pl.BlockSpec(memory_space=pltpu.HBM)
    out = pl.pallas_call(
        kernel,
        out_shape=jax.ShapeDtypeStruct((B, M), A_x.dtype),
        in_specs=[hbm] * 11,
        out_specs=pl.BlockSpec(memory_space=pltpu.VMEM),
        scratch_shapes=[
            pltpu.VMEM((B, M), BF16),
            pltpu.VMEM((M,), BF16),
            pltpu.VMEM((M * H, D), BF16),
            pltpu.VMEM((DC * H, D), BF16),
            pltpu.VMEM((DC * H, D), BF16),
            pltpu.VMEM((H * D, M), BF16),
            pltpu.VMEM((M, H * D), BF16),
            pltpu.VMEM((H * D, M), BF16),
            pltpu.VMEM((2, SK, DC), BF16),
            pltpu.VMEM((2, HKV, W, D), BF16),
            pltpu.VMEM((2, HKV, W, D), BF16),
            pltpu.VMEM((H, B, D), F32),
            pltpu.VMEM((B, H, DC), F32),
            pltpu.VMEM((B, H, DC), F32),
            pltpu.VMEM((B, H, D), F32),
            pltpu.VMEM((B, H, D), F32),
            pltpu.SemaphoreType.DMA((N_SEMS,)),
        ],
        compiler_params=pltpu.CompilerParams(vmem_limit_bytes=96 * 1024 * 1024),
    )(
        A_x.reshape(B, M), gate_w, A_c_kv,
        A_w_q.reshape(M * H, D), A_w_uk.reshape(DC * H, D), A_w_uv.reshape(DC * H, D),
        A_w_o.reshape(H * D, M), B_k_cache, B_v_cache, B_wq, B_wo,
    )
    return out.reshape(B, Sq, M)
```

```python
import jax
import jax.numpy as jnp
from jax import lax
import jax.experimental.pallas as pl
import jax.experimental.pallas.tpu as pltpu

F32, BF16 = jnp.float32, jnp.bfloat16
N_SEMS = 3

_NN = (((1,), (0,)), ((), ()))
_NT = (((1,), (1,)), ((), ()))


def _mm(a, b, dims=_NN):
    return lax.dot_general(a, b, dims, preferred_element_type=F32)


def _head_pair(w32_ref, j, rows, heads):
    w = w32_ref[pl.ds(j, rows, stride=heads // 2), :]
    even = pltpu.bitcast(w << 16, F32).astype(BF16)
    odd = pltpu.bitcast(w & jnp.uint32(0xFFFF0000), F32).astype(BF16)
    return even, odd


def _as_words(src_ref, dst_ref, step_rows=2048):
    half = step_rows // 2

    def step(i, carry):
        rows = src_ref[pl.ds(pl.multiple_of(i * step_rows, step_rows), step_rows), :]
        dst_ref[pl.ds(pl.multiple_of(i * half, half), half), :] = pltpu.bitcast(rows, jnp.uint32)
        return carry

    lax.fori_loop(0, src_ref.shape[0] // step_rows, step, 0)


def _exp_max(s):
    e = jnp.exp(s - jnp.max(s, axis=-1, keepdims=True))
    return e, jnp.sum(e, axis=-1, keepdims=True)


def _chunks(total):
    sizes = [total // 4] * 3 + [total // 8, total // 16, total // 32, total // 32]
    assert sum(sizes) == total and all(s % 128 == 0 for s in sizes), sizes
    return sizes


@jax.jit
def pallas_gated_mix__compressed_kv_cla__sliding_block_cached__decode_kernel(
    A_x: jax.Array,
    A_c_kv: jax.Array,
    A_w_q: jax.Array,
    A_w_uk: jax.Array,
    A_w_uv: jax.Array,
    A_w_o: jax.Array,
    B_x: jax.Array,
    B_k_cache: jax.Array,
    B_v_cache: jax.Array,
    B_wq: jax.Array,
    B_wo: jax.Array,
    gate_w: jax.Array,
):
    del B_x
    B, Sq, M = A_x.shape
    _, SK, DC = A_c_kv.shape
    _, H, D = A_w_q.shape
    _, HKV, SKB, _ = B_k_cache.shape
    W = min(4096, max(256, SKB // 4))
    REP = H // HKV
    assert Sq == 1 and B == 8 and REP == 4 and D == 128, (Sq, B, REP, D)
    scale = float(D) ** -0.5
    wob_rows = _chunks(H * D)
    wob_offs = [sum(wob_rows[:i]) for i in range(len(wob_rows))]

    def kernel(x_hbm, gw_hbm, c_hbm, wq_hbm, wuk_hbm, wuv_hbm, wo_hbm,
               k_hbm, v_hbm, wqb_hbm, wob_hbm,
               o_ref,
               x_v, gw_v, wq_v, wuk_v, wuv_v, wo_v, wqb_v, wob_v, c_v, k_v, v_v,
               q_s, qlat_s, clat_s, qb_s, ob_s, w32_s, sems):

        def c_copy(b):
            return pltpu.make_async_copy(c_hbm.at[b], c_v.at[b % 2], sems.at[0])

        def k_copy(b):
            return pltpu.make_async_copy(
                k_hbm.at[b, :, pl.ds(SKB - W, W), :], k_v.at[b % 2], sems.at[1])

        def v_copy(b):
            return pltpu.make_async_copy(
                v_hbm.at[b, :, pl.ds(SKB - W, W), :], v_v.at[b % 2], sems.at[2])

        x_cp = pltpu.make_async_copy(x_hbm, x_v, sems.at[0])
        gw_cp = pltpu.make_async_copy(gw_hbm, gw_v, sems.at[0])
        wq_cp = pltpu.make_async_copy(wq_hbm, wq_v, sems.at[0])
        wuk_cp = pltpu.make_async_copy(wuk_hbm, wuk_v, sems.at[1])
        wqb_cp = pltpu.make_async_copy(wqb_hbm, wqb_v, sems.at[2])
        tail = [pltpu.make_async_copy(wuv_hbm, wuv_v, sems.at[0]),
                pltpu.make_async_copy(wo_hbm, wo_v, sems.at[1])]
        tail += [pltpu.make_async_copy(wob_hbm.at[pl.ds(o, n)], wob_v.at[pl.ds(o, n)],
                                       sems.at[(2 + i) % N_SEMS])
                 for i, (o, n) in enumerate(zip(wob_offs, wob_rows))]

        def tail_wait(t):
            tail[t].wait()
            if t + N_SEMS < len(tail):
                tail[t + N_SEMS].start()

        wq_cp.start()
        x_cp.start()
        gw_cp.start()
        wuk_cp.start()
        wqb_cp.start()

        x_cp.wait()
        gw_cp.wait()
        wq_cp.wait()
        c_copy(0).start()
        x = x_v[...]

        _as_words(wq_v, w32_s)
        for j in range(H // 2):
            for h, w in zip((2 * j, 2 * j + 1), _head_pair(w32_s, j, M, H)):
                q_s[h] = _mm(x, w)

        wuk_cp.wait()
        k_copy(0).start()
        _as_words(wuk_v, w32_s)
        for j in range(H // 2):
            for h, w in zip((2 * j, 2 * j + 1), _head_pair(w32_s, j, DC, H)):
                qlat_s[:, h, :] = _mm(q_s[h].astype(BF16), w, _NT) * scale

        wqb_cp.wait()
        v_copy(0).start()
        for h in range(H):
            qb_s[:, h, :] = _mm(x, wqb_v[:, h * D:(h + 1) * D])

        row_w = lax.broadcasted_iota(jnp.int32, (2 * REP, W), 0)
        row_d = lax.broadcasted_iota(jnp.int32, (2 * REP, D), 0)

        def start_next(b, copy, last):
            @pl.when(b + 1 < B)
            def _():
                copy(b + 1).start()

            @pl.when(b + 1 == B)
            def _():
                last.start()

        def per_batch(b, carry):
            slot = b % 2

            c_copy(b).wait()
            start_next(b, c_copy, tail[0])
            c = c_v.at[slot]
            e, l = _exp_max(_mm(qlat_s[b].astype(BF16), c[...], _NT))
            clat_s[b] = _mm(e.astype(BF16), c[...]) / l

            k_copy(b).wait()
            start_next(b, k_copy, tail[1])
            v_copy(b).wait()
            start_next(b, v_copy, tail[2])
            qb = (qb_s[b].astype(BF16).astype(F32) * scale).astype(BF16)
            for i in range(HKV // 2):
                qi = qb[2 * REP * i:2 * REP * (i + 1), :]
                s = jnp.where(row_w < REP,
                              _mm(qi, k_v[slot, 2 * i], _NT),
                              _mm(qi, k_v[slot, 2 * i + 1], _NT))
                eb, lb = _exp_max(s)
                p = eb.astype(BF16)
                o = jnp.where(row_d < REP,
                              _mm(p, v_v[slot, 2 * i]),
                              _mm(p, v_v[slot, 2 * i + 1]))
                ob_s[b, 2 * REP * i:2 * REP * (i + 1), :] = o / lb
            return carry

        lax.fori_loop(0, B, per_batch, 0)

        tail_wait(0)
        _as_words(wuv_v, w32_s)
        ctx = []
        for j in range(H // 2):
            for h, w in zip((2 * j, 2 * j + 1), _head_pair(w32_s, j, DC, H)):
                ctx.append(_mm(clat_s[:, h, :].astype(BF16), w).astype(BF16))
        ctx = jnp.concatenate(ctx, axis=1)
        ob = jnp.concatenate([ob_s[:, h, :].astype(BF16) for h in range(H)], axis=1)
        g = jax.nn.sigmoid(jnp.sum(x.astype(F32) * gw_v[...].astype(F32).reshape(1, M),
                                   axis=-1, keepdims=True))
        tail_wait(1)
        ga = g * _mm(ctx, wo_v[...])

        bo = jnp.zeros((B, M), F32)
        for i, (o, n) in enumerate(zip(wob_offs, wob_rows)):
            tail_wait(2 + i)
            bo = bo + _mm(ob[:, o:o + n], wob_v[pl.ds(o, n), :])

        o_ref[...] = (ga + (1.0 - g) * bo).astype(o_ref.dtype)

    hbm = pl.BlockSpec(memory_space=pltpu.HBM)
    out = pl.pallas_call(
        kernel,
        out_shape=jax.ShapeDtypeStruct((B, M), A_x.dtype),
        in_specs=[hbm] * 11,
        out_specs=pl.BlockSpec(memory_space=pltpu.VMEM),
        scratch_shapes=[
            pltpu.VMEM((B, M), BF16),
            pltpu.VMEM((M,), BF16),
            pltpu.VMEM((M * H, D), BF16),
            pltpu.VMEM((DC * H, D), BF16),
            pltpu.VMEM((DC * H, D), BF16),
            pltpu.VMEM((H * D, M), BF16),
            pltpu.VMEM((M, H * D), BF16),
            pltpu.VMEM((H * D, M), BF16),
            pltpu.VMEM((2, SK, DC), BF16),
            pltpu.VMEM((2, HKV, W, D), BF16),
            pltpu.VMEM((2, HKV, W, D), BF16),
            pltpu.VMEM((H, B, D), F32),
            pltpu.VMEM((B, H, DC), F32),
            pltpu.VMEM((B, H, DC), F32),
            pltpu.VMEM((B, H, D), F32),
            pltpu.VMEM((B, H, D), F32),
            pltpu.VMEM((M * H // 2, D), jnp.uint32),
            pltpu.SemaphoreType.DMA((N_SEMS,)),
        ],
        compiler_params=pltpu.CompilerParams(vmem_limit_bytes=96 * 1024 * 1024),
    )(
        A_x.reshape(B, M), gate_w, A_c_kv,
        A_w_q.reshape(M * H, D), A_w_uk.reshape(DC * H, D), A_w_uv.reshape(DC * H, D),
        A_w_o.reshape(H * D, M), B_k_cache, B_v_cache, B_wq, B_wo,
    )
    return out.reshape(B, Sq, M)
```
